```python
import jax
import jax.numpy as jnp

def _softmax(x, axis=-1):
    return jax.nn.softmax(x, axis=axis)
def _gelu(x):
    return jax.nn.gelu(x, approximate=True)
def _silu(x):
    return jax.nn.silu(x)
def _sigmoid(x):
    return jax.nn.sigmoid(x)
def _layernorm(x, axis=-1, eps=1e-5):
    m = jnp.mean(x, axis=axis, keepdims=True)
    v = jnp.var(x, axis=axis, keepdims=True)
    return (x - m) / jnp.sqrt(v + eps)
def _scatter_add(tgt, idx, src, axis=0):
    return tgt.at[idx].add(src)
def _segment_sum(src, seg, n):
    return jax.ops.segment_sum(src, seg, n)
class _Rng:
    def __init__(self, key):
        self._k = key
    def _next(self):
        self._k, sub = jax.random.split(self._k)
        return sub
    def normal(self, shape):
        return jax.random.normal(self._next(), shape, dtype=jnp.bfloat16)
    def randint(self, lo, hi, shape):
        return jax.random.randint(self._next(), shape, lo, hi, dtype=jnp.int32)
    def uniform(self, shape, lo=0.0, hi=1.0):
        return jax.random.uniform(self._next(), shape, jnp.bfloat16, lo, hi)
    def permutation(self, n):
        return jax.random.permutation(self._next(), n)


kernel_name = 'interleave_layers__sliding_local_dilated__glu_gated_geglu__prompt'

def setup_inputs():
    _rng = _Rng(jax.random.key(int.from_bytes(__import__("os").urandom(4), "little")))
    _w = (lambda a: (lambda t: t.astype(jnp.bfloat16) if jnp.issubdtype(t.dtype, jnp.floating) else t)(jnp.asarray(a)))
    def _A_setup():
        B, S, D = 1, 2048, 576
        return {
            "x": _w((lambda *s: _rng.normal(s) * 0.05)(B, S, D)),
            "wqkv": _w((lambda *s: _rng.normal(s) * 0.05)(D, 3 * D)),
            "wo": _w((lambda *s: _rng.normal(s) * 0.05)(D, D)),
        }
    _A_in = _A_setup()

    def _B_setup():
        B, S, Dm, Df = 1, 2048, 576, 4608
        return {
            "x": _w((lambda *s: _rng.normal(s) * 0.05)(B, S, Dm)),
            "w_gate": _w((lambda *s: _rng.normal(s) * 0.05)(Dm, Df) * (Dm ** -0.5)),
            "w_up": _w((lambda *s: _rng.normal(s) * 0.05)(Dm, Df) * (Dm ** -0.5)),
            "w_down": _w((lambda *s: _rng.normal(s) * 0.05)(Df, Dm) * (Df ** -0.5)),
        }
    _B_in = _B_setup()

    return {
        "A_x": _A_in["x"],
        "A_wqkv": _A_in["wqkv"],
        "A_wo": _A_in["wo"],
        "B_x": _B_in["x"],
        "B_w_gate": _B_in["w_gate"],
        "B_w_up": _B_in["w_up"],
        "B_w_down": _B_in["w_down"],
    }

def reference(A_x, A_wqkv, A_wo, B_x, B_w_gate, B_w_up, B_w_down):
    def _A_ref(x, wqkv, wo):
        B, S, D = x.shape
        H = 32; Dh = D // H
        W, dil = 8, 2
        qkv = (lambda x, *d: x.transpose(*d))((x @ wqkv).reshape(B, S, 3, H, Dh), 2, 0, 3, 1, 4)
        q, k, v = qkv[0], qkv[1], qkv[2]
        scale = Dh ** -0.5
        pos = jnp.arange(S)
        off = jnp.arange(W) * dil
        idx = pos[:, None] - off[None, :]
        mask = idx >= 0
        idx_c = jnp.where(mask, idx, 0).reshape(-1)
        kg = k[:, :, idx_c, :].reshape(B, H, S, W, Dh)
        vg = v[:, :, idx_c, :].reshape(B, H, S, W, Dh)
        logits = jnp.einsum("bhsd,bhswd->bhsw", q, kg) * scale
        logits = jnp.where(mask[None, None, :, :], logits, -1e9)
        attn = _softmax(logits, axis=-1)
        o = jnp.einsum("bhsw,bhswd->bhsd", attn, vg)
        return (lambda x, *d: x.transpose(*d))(o, 0, 2, 1, 3).reshape(B, S, D) @ wo

    def _B_ref(x, w_gate, w_up, w_down):
        g = jnp.einsum("bsd,df->bsf", x, w_gate)
        u = jnp.einsum("bsd,df->bsf", x, w_up)
        h = _gelu(g) * u
        return jnp.einsum("bsf,fd->bsd", h, w_down)

    x = A_x
    x = x + _A_ref(_layernorm(x, axis=-1), A_wqkv, A_wo)
    x = x + _B_ref(_layernorm(x, axis=-1), B_w_gate, B_w_up, B_w_down)
    x = x + _A_ref(_layernorm(x, axis=-1), A_wqkv, A_wo)
    x = x + _B_ref(_layernorm(x, axis=-1), B_w_gate, B_w_up, B_w_down)
    return x
```

```python
import functools

import jax
import jax.numpy as jnp
import numpy as np
import jax.experimental.pallas as pl
import jax.experimental.pallas.tpu as pltpu

S, D, F = 2048, 576, 4608
H, DH = 32, 18
WIN, DIL = 8, 2
EPS = 1e-5
TB = 512
FC = 512
LANES = 128
NT5 = -(-D // LANES)
bf16, f32 = jnp.bfloat16, jnp.float32
NN = (((1,), (0,)), ((), ()))
TN = (((0,), (0,)), ((), ()))


def _dot(a, b, dims=NN):
    return jax.lax.dot_general(a, b, dims, preferred_element_type=f32)


def _layernorm_t(x):
    m = jnp.mean(x, axis=0, keepdims=True)
    xc = x - m
    v = jnp.mean(xc * xc, axis=0, keepdims=True)
    return xc / jnp.sqrt(v + EPS)


def _geglu(g, u):
    c0 = np.float32(np.sqrt(2.0 / np.pi))
    c1 = np.float32(0.044715)
    inner = c0 * (g + c1 * (g * g * g))
    return (np.float32(0.5) * g * (np.float32(1.0) + jnp.tanh(inner))) * u


def _kernel(x_hbm, wqkv_hbm, wo_hbm, wg_hbm, wu_hbm, wd_hbm, out_hbm,
            x_v, wqkv_v, wo_v, wg_v, wu_v, wd_v,
            tmp, wq_t, wo_t, res, xn, q_s, k_s, v_s, o_s, out_v, sems):
    cp_x = pltpu.make_async_copy(x_hbm, x_v, sems.at[0])
    cp_qkv = pltpu.make_async_copy(wqkv_hbm, wqkv_v, sems.at[1])
    cp_o = pltpu.make_async_copy(wo_hbm, wo_v, sems.at[2])
    cp_g = pltpu.make_async_copy(wg_hbm, wg_v, sems.at[3])
    cp_u = pltpu.make_async_copy(wu_hbm, wu_v, sems.at[4])
    cp_d = pltpu.make_async_copy(wd_hbm, wd_v, sems.at[5])
    for c in (cp_qkv, cp_x, cp_o, cp_g, cp_u, cp_d):
        c.start()

    cp_qkv.wait()
    for j in range(NT5):
        kw = min(LANES, D - j * LANES)
        tmp[j, :, 0:kw] = wqkv_v[j * LANES:j * LANES + kw, :].astype(f32).T
    for p in range(3):
        for d in range(DH):
            r = p * D + d * H
            for j in range(NT5):
                kw = min(LANES, D - j * LANES)
                wq_t[r:r + H, j * LANES:j * LANES + kw] = tmp[
                    j, pl.ds(p * D + d, H, stride=DH), 0:kw].astype(bf16)
    cp_o.wait()
    for j in range(NT5):
        nw = min(LANES, D - j * LANES)
        tmp[j, 0:D, 0:nw] = wo_v[:, j * LANES:j * LANES + nw].astype(f32)
        perm = jnp.concatenate(
            [tmp[j, pl.ds(d, H, stride=DH), 0:nw] for d in range(DH)], axis=0)
        wo_t[j * LANES:j * LANES + nw, :] = perm.T.astype(bf16)

    cp_x.wait()
    res[...] = x_v[...].astype(f32)

    scale = np.float32(DH ** -0.5)

    def attention(t):
        t0 = pl.multiple_of(t * TB, TB)
        xn[...] = _layernorm_t(res[:, pl.ds(t0, TB)]).astype(bf16)
        qkv = _dot(wq_t[...], xn[...])
        q_s[...] = qkv[0:D] * scale
        k_s[:, LANES:] = qkv[D:2 * D]
        v_s[:, LANES:] = qkv[2 * D:3 * D]
        pos = t0 + jax.lax.broadcasted_iota(jnp.int32, (8, TB), 1)

        def head_group(hg, carry):
            r0 = pl.multiple_of(hg * 8, 8)
            logits = [None] * WIN
            for d in range(DH):
                q = q_s[pl.ds(d * H + r0, 8), :]
                k = k_s[pl.ds(d * H + r0, 8), :]
                for w in range(WIN):
                    kw = k if w == 0 else pltpu.roll(k, w * DIL, 1)
                    prod = q * kw[:, LANES:]
                    logits[w] = prod if d == 0 else logits[w] + prod
            for w in range(1, WIN):
                logits[w] = jnp.where(pos >= w * DIL, logits[w], np.float32(-1e9))
            m = functools.reduce(jnp.maximum, logits)
            e = [jnp.exp(l - m) for l in logits]
            inv = 1.0 / functools.reduce(jnp.add, e)
            a = [x * inv for x in e]
            for d in range(DH):
                v = v_s[pl.ds(d * H + r0, 8), :]
                o = None
                for w in range(WIN):
                    vw = v if w == 0 else pltpu.roll(v, w * DIL, 1)
                    term = a[w] * vw[:, LANES:]
                    o = term if o is None else o + term
                o_s[pl.ds(d * H + r0, 8), :] = o
            return carry

        jax.lax.fori_loop(0, H // 8, head_group, 0)
        res[:, pl.ds(t0, TB)] += _dot(wo_t[...], o_s[...].astype(bf16))
        k_s[:, 0:LANES] = k_s[:, TB:TB + LANES]
        v_s[:, 0:LANES] = v_s[:, TB:TB + LANES]

    def ffn(t):
        t0 = pl.multiple_of(t * TB, TB)
        xn[...] = _layernorm_t(res[:, pl.ds(t0, TB)]).astype(bf16)

        def chunk(c, carry):
            c0 = pl.multiple_of(c * FC, FC)
            g = _dot(wg_v[:, pl.ds(c0, FC)], xn[...], TN)
            u = _dot(wu_v[:, pl.ds(c0, FC)], xn[...], TN)
            h = _geglu(g, u).astype(bf16)
            res[:, pl.ds(t0, TB)] += _dot(wd_v[:, pl.ds(c0, FC)], h)
            return carry

        jax.lax.fori_loop(0, F // FC, chunk, 0)

    for layer in range(2):
        k_s[:, 0:LANES] = jnp.zeros((D, LANES), f32)
        v_s[:, 0:LANES] = jnp.zeros((D, LANES), f32)

        def block(t, carry):
            attention(t)
            ffn(t)
            return carry

        if layer == 0:
            cp_g.wait()
            cp_u.wait()
            cp_d.wait()
        jax.lax.fori_loop(0, S // TB, block, 0)

    out_v[...] = res[...].astype(bf16)
    cp_out = pltpu.make_async_copy(out_v, out_hbm, sems.at[6])
    cp_out.start()
    cp_out.wait()


@jax.jit
def pallas_interleave_layers__sliding_local_dilated__glu_gated_geglu__prompt_kernel(
    A_x: jax.Array,
    A_wqkv: jax.Array,
    A_wo: jax.Array,
    B_x: jax.Array,
    B_w_gate: jax.Array,
    B_w_up: jax.Array,
    B_w_down: jax.Array,
):
    del B_x
    x_t = A_x.reshape(S, D).T
    wd_t = B_w_down.T
    hbm = pl.BlockSpec(memory_space=pl.ANY)
    out_t = pl.pallas_call(
        _kernel,
        out_shape=jax.ShapeDtypeStruct((D, S), bf16),
        in_specs=[hbm] * 6,
        out_specs=hbm,
        scratch_shapes=[
            pltpu.VMEM((D, S), bf16),
            pltpu.VMEM((D, 3 * D), bf16),
            pltpu.VMEM((D, D), bf16),
            pltpu.VMEM((D, F), bf16),
            pltpu.VMEM((D, F), bf16),
            pltpu.VMEM((D, F), bf16),
            pltpu.VMEM((NT5, 3 * D, LANES), f32),
            pltpu.VMEM((3 * D, D), bf16),
            pltpu.VMEM((D, D), bf16),
            pltpu.VMEM((D, S), f32),
            pltpu.VMEM((D, TB), bf16),
            pltpu.VMEM((D, TB), f32),
            pltpu.VMEM((D, LANES + TB), f32),
            pltpu.VMEM((D, LANES + TB), f32),
            pltpu.VMEM((D, TB), f32),
            pltpu.VMEM((D, S), bf16),
            pltpu.SemaphoreType.DMA((7,)),
        ],
        compiler_params=pltpu.CompilerParams(vmem_limit_bytes=100 * 1024 * 1024),
        name="interleave_attn_geglu",
    )(x_t, A_wqkv, A_wo, B_w_gate, B_w_up, wd_t)
    return out_t.T.reshape(1, S, D)
```

```python
import functools, os

import jax
import jax.numpy as jnp
import numpy as np
import jax.experimental.pallas as pl
import jax.experimental.pallas.tpu as pltpu

S, D, F = 2048, 576, 4608
H, DH = 32, 18
WIN, DIL = 8, 2
EPS = 1e-5
TB = int(os.environ.get("TB", 512))
NB = S // TB
NBLK = 2 * NB
HG = 8
NG = H // HG
FC = F // NG
GR = HG * DH
LANES = 128
NT5 = -(-D // LANES)
bf16, f32 = jnp.bfloat16, jnp.float32
NN = (((1,), (0,)), ((), ()))
ABL = os.environ.get('ABL', '')


def _dot(a, b, dims=NN):
    return jax.lax.dot_general(a, b, dims, preferred_element_type=f32)


def _layernorm_t(x):
    m = jnp.mean(x, axis=0, keepdims=True)
    xc = x - m
    v = jnp.mean(xc * xc, axis=0, keepdims=True)
    return xc * jax.lax.rsqrt(v + EPS)


def _geglu(g, u):
    c0 = np.float32(np.sqrt(2.0 / np.pi))
    c1 = np.float32(np.sqrt(2.0 / np.pi) * 0.044715)
    inner = g * (c0 + c1 * (g * g))
    return (g * u) * (np.float32(0.5) + np.float32(0.5) * jnp.tanh(inner))


def _kernel(x_hbm, wqkv_hbm, wo_hbm, wg_hbm, wu_hbm, wd_hbm, out_hbm,
            x_v, wqkv_v, wo_v, wg_v, wu_v, wd_v,
            tmp, wq_t, wo_t, wg_t, wu_t, res, xn1, xn2, q_s, k_s, v_s, o_s, out_v,
            sem_x, sem_a, sem_w, sem_o):
    def cols(i, n):
        return pl.ds(i * n if isinstance(i, int) else pl.multiple_of(i * n, LANES), n)

    cp_x = [pltpu.make_async_copy(x_hbm.at[:, cols(t, TB)], x_v.at[:, cols(t, TB)], sem_x.at[t])
            for t in range(NB)]
    cp_qkv = pltpu.make_async_copy(wqkv_hbm, wqkv_v, sem_a.at[0])
    cp_o = pltpu.make_async_copy(wo_hbm, wo_v, sem_a.at[1])

    def cp_w(c):
        return [pltpu.make_async_copy(src.at[:, cols(c, FC)], dst.at[:, cols(c, FC)], sem_w.at[j, c])
                for j, (src, dst) in enumerate(((wg_hbm, wg_v), (wu_hbm, wu_v), (wd_hbm, wd_v)))]

    def cp_out(t):
        return pltpu.make_async_copy(out_v.at[:, cols(t, TB)], out_hbm.at[:, cols(t, TB)], sem_o.at[t])

    cp_x[0].start()
    cp_qkv.start()

    scale = np.float32(DH ** -0.5)

    def prep_qkv():
        for j in range(NT5):
            kw = min(LANES, D - j * LANES)
            tmp[j, :, 0:kw] = wqkv_v[j * LANES:j * LANES + kw, :].astype(f32).T
        for g in range(NG):
            for p in range(3):
                for d in range(0, DH, 2):
                    r = (g * 3 + p) * GR + d * HG
                    src = p * D + g * GR + d
                    for j in range(NT5):
                        kw = min(LANES, D - j * LANES)
                        two = jnp.concatenate(
                            [tmp[j, pl.ds(src + e, HG, stride=DH), 0:kw] for e in range(2)], axis=0)
                        wq_t[r:r + 2 * HG, j * LANES:j * LANES + kw] = two.astype(bf16)

    def prep_wo():
        for j in range(NT5):
            nw = min(LANES, D - j * LANES)
            tmp[j, 0:D, 0:nw] = wo_v[:, j * LANES:j * LANES + nw].astype(f32)
            perm = jnp.concatenate(
                [tmp[j, pl.ds(g * GR + d, HG, stride=DH), 0:nw] for g in range(NG) for d in range(DH)],
                axis=0)
            wo_t[j * LANES:j * LANES + nw, :] = perm.T.astype(bf16)

    def prep_ffn(c):
        if 'p' in ABL: return
        wg_t[pl.ds(c * FC, FC), :] = wg_v[:, cols(c, FC)].T
        wu_t[pl.ds(c * FC, FC), :] = wu_v[:, cols(c, FC)].T

    def ln1(b):
        if 'l' in ABL: return
        xn1[...] = _layernorm_t(res[:, cols(b % NB, TB)]).astype(bf16)

    def qkv(b, g):
        if 'q' in ABL: return
        slot = b % 2
        qkv = _dot(wq_t[pl.ds(pl.multiple_of(g * 3 * GR, 16), 3 * GR), :], xn1[...])
        rows = pl.ds(pl.multiple_of(g * GR, 8), GR)
        keep = (b % NB) > 0
        k_s[slot, rows, 0:LANES] = jnp.where(keep, k_s[1 - slot, rows, TB:TB + LANES], 0.0)
        v_s[slot, rows, 0:LANES] = jnp.where(keep, v_s[1 - slot, rows, TB:TB + LANES], 0.0)
        q_s[slot, rows, :] = qkv[0:GR] * scale
        k_s[slot, rows, LANES:] = qkv[GR:2 * GR]
        v_s[slot, rows, LANES:] = qkv[2 * GR:3 * GR]

    def heads(b, g):
        if 'h' in ABL: return
        slot = b % 2
        pos = (b % NB) * TB + jax.lax.broadcasted_iota(jnp.int32, (HG, TB), 1)
        r0 = pl.multiple_of(g * GR, 8)
        logits = [None] * WIN
        for d in range(DH):
            q = q_s[slot, pl.ds(r0 + d * HG, HG), :]
            k = k_s[slot, pl.ds(r0 + d * HG, HG), :]
            for w in range(WIN):
                kw = k if w == 0 else pltpu.roll(k, w * DIL, 1)
                prod = q * kw[:, LANES:]
                logits[w] = prod if d == 0 else logits[w] + prod
        for w in range(1, WIN):
            logits[w] = jnp.where(pos >= w * DIL, logits[w], np.float32(-1e9))
        m = functools.reduce(jnp.maximum, logits)
        e = [jnp.exp(l - m) for l in logits]
        inv = 1.0 / functools.reduce(jnp.add, e)
        a = [x * inv for x in e]
        for d in range(DH):
            v = v_s[slot, pl.ds(r0 + d * HG, HG), :]
            o = None
            for w in range(WIN):
                vw = v if w == 0 else pltpu.roll(v, w * DIL, 1)
                term = a[w] * vw[:, LANES:]
                o = term if o is None else o + term
            o_s[pl.ds(r0 + d * HG, HG), :] = o

    def attn_out(b):
        if 'o' in ABL: return
        blk = cols(b % NB, TB)
        x1 = res[:, blk] + _dot(wo_t[...], o_s[...].astype(bf16))
        res[:, blk] = x1
        xn2[...] = _layernorm_t(x1).astype(bf16)

    def ffn(b, c):
        if 'f' in ABL: return
        blk = cols(b % NB, TB)
        SUB = int(os.environ.get('SUB', 1)); FS = FC // SUB
        acc = None
        for s in range(SUB):
            rows = pl.ds(pl.multiple_of(c * FC + s * FS, LANES), FS)
            g = _dot(wg_t[rows, :], xn2[...])
            u = _dot(wu_t[rows, :], xn2[...])
            h = _geglu(g, u).astype(bf16)
            d = _dot(wd_v[:, rows], h)
            acc = d if acc is None else acc + d
        res[:, blk] += acc

    def emit(b):
        t = b - NB
        out_v[:, cols(t, TB)] = res[:, cols(t, TB)].astype(bf16)
        cp_out(t).start()

    def loop(n, body, lo=0):
        jax.lax.fori_loop(lo, n, lambda i, carry: (body(i), carry)[1], 0)

    k_s[1, :, TB:] = jnp.zeros((D, LANES), f32)
    v_s[1, :, TB:] = jnp.zeros((D, LANES), f32)

    def load_x(t):
        cp_x[t].wait()
        res[:, cols(t, TB)] = x_v[:, cols(t, TB)].astype(f32)

    load_x(0)
    ln1(0)
    cp_qkv.wait()
    cp_x[1].start()
    cp_o.start()
    for cp in cp_w(0):
        cp.start()
    prep_qkv()
    loop(NG, lambda g: qkv(0, g))
    for cp in cp_x[2:] + cp_w(1):
        cp.start()
    load_x(1)
    ln1(1)
    loop(NG, lambda g: (heads(0, g), qkv(1, g)))
    for cp in cp_w(2):
        cp.start()
    cp_o.wait()
    prep_wo()
    for t in range(2, NB):
        load_x(t)
    for cp in cp_w(0):
        cp.wait()
    prep_ffn(0)
    ln1(2)
    attn_out(0)
    for cp in cp_w(3):
        cp.start()

    def first(c):
        @pl.when(c + 1 < NG)
        def _():
            for cp in cp_w(c + 1):
                cp.wait()
        ffn(0, c)
        heads(1, c)
        qkv(2, c)
        if NG > 1:
            prep_ffn(jnp.minimum(c + 1, NG - 1))
    loop(NG - 1, first)
    ffn(0, NG - 1)
    heads(1, NG - 1)
    qkv(2, NG - 1)
    ln1(3)
    attn_out(1)

    def step(i):
        loop(NG, lambda c: (ffn(i, c), heads(i + 1, c), qkv(i + 2, c)))

        @pl.when((i >= NB) & (i < NBLK - 2))
        def _():
            emit(i)
        ln1(jnp.minimum(i + 3, NBLK - 1))
        attn_out(i + 1)
    loop(NBLK - 2 + int(os.environ.get('EXTRA', 0)), step, lo=1)

    i = NBLK - 2
    loop(NG, lambda c: (ffn(i, c), heads(i + 1, c)))
    emit(i)
    attn_out(i + 1)
    i = NBLK - 1
    loop(NG, lambda c: ffn(i, c))
    emit(i)
    for t in range(NB):
        cp_out(t).wait()


@jax.jit
def pallas_interleave_layers__sliding_local_dilated__glu_gated_geglu__prompt_kernel(
    A_x: jax.Array,
    A_wqkv: jax.Array,
    A_wo: jax.Array,
    B_x: jax.Array,
    B_w_gate: jax.Array,
    B_w_up: jax.Array,
    B_w_down: jax.Array,
):
    del B_x
    x_t = A_x.reshape(S, D).T
    wd_t = B_w_down.T
    hbm = pl.BlockSpec(memory_space=pl.ANY)
    out_t = pl.pallas_call(
        _kernel,
        out_shape=jax.ShapeDtypeStruct((D, S), bf16),
        in_specs=[hbm] * 6,
        out_specs=hbm,
        scratch_shapes=[
            pltpu.VMEM((D, S), bf16),
            pltpu.VMEM((D, 3 * D), bf16),
            pltpu.VMEM((D, D), bf16),
            pltpu.VMEM((D, F), bf16),
            pltpu.VMEM((D, F), bf16),
            pltpu.VMEM((D, F), bf16),
            pltpu.VMEM((NT5, 3 * D, LANES), f32),
            pltpu.VMEM((3 * D, D), bf16),
            pltpu.VMEM((D, D), bf16),
            pltpu.VMEM((F, D), bf16),
            pltpu.VMEM((F, D), bf16),
            pltpu.VMEM((D, S), f32),
            pltpu.VMEM((D, TB), bf16),
            pltpu.VMEM((D, TB), bf16),
            pltpu.VMEM((2, D, TB), f32),
            pltpu.VMEM((2, D, LANES + TB), f32),
            pltpu.VMEM((2, D, LANES + TB), f32),
            pltpu.VMEM((D, TB), f32),
            pltpu.VMEM((D, S), bf16),
            pltpu.SemaphoreType.DMA((NB,)),
            pltpu.SemaphoreType.DMA((2,)),
            pltpu.SemaphoreType.DMA((3, NG)),
            pltpu.SemaphoreType.DMA((NB,)),
        ],
        compiler_params=pltpu.CompilerParams(vmem_limit_bytes=100 * 1024 * 1024),
        name="interleave_attn_geglu",
    )(x_t, A_wqkv, A_wo, B_w_gate, B_w_up, wd_t)
    return out_t.T.reshape(1, S, D)
```

```python
import functools, os

import jax
import jax.numpy as jnp
import numpy as np
import jax.experimental.pallas as pl
import jax.experimental.pallas.tpu as pltpu

S, D, F = 2048, 576, 4608
H, DH = 32, 18
WIN, DIL = 8, 2
EPS = 1e-5
LANES = 128
TB = 256
TH = TB // 2
NB = S // TB
NBLK = 2 * NB
HG = 8
NG = H // HG
GR = HG * DH
NT5 = -(-D // LANES)
F2, D2 = F // 2, D // 2
KH = 256
KT = D - 2 * KH
NS = int(os.environ.get('NS', 6))
FS = F2 // NS
DSUB = int(os.environ.get('DSUB', 6))
PACK = int(os.environ.get('PACK', 1))
HPOS = [int(c) for c in os.environ.get('HPOS', '0123')]
bf16, f32 = jnp.bfloat16, jnp.float32
NN = (((1,), (0,)), ((), ()))
ABL = os.environ.get('ABL', '')


def _dot(a, b):
    return jax.lax.dot_general(a, b, NN, preferred_element_type=f32)


def _layernorm_t(x):
    m = jnp.mean(x, axis=0, keepdims=True)
    xc = x - m
    v = jnp.mean(xc * xc, axis=0, keepdims=True)
    return xc * jax.lax.rsqrt(v + EPS)


def _geglu(g, u):
    c0 = np.float32(np.sqrt(2.0 / np.pi))
    c1 = np.float32(np.sqrt(2.0 / np.pi) * 0.044715)
    inner = g * (c0 + c1 * (g * g))
    return (g * u) * (np.float32(0.5) + np.float32(0.5) * jnp.tanh(inner))


def _strassen_lhs(a11, a12, a21, a22):
    return [a11 + a22, a21 + a22, a11, a22, a11 + a12, a21 - a11, a12 - a22]


def _strassen_rhs(b11, b12, b21, b22):
    return [b11 + b22, b11, b12 - b22, b21 - b11, b22, b11 + b12, b21 + b22]


def _strassen_out(m):
    return (m[0] + m[3] - m[4] + m[6], m[2] + m[4], m[1] + m[3], m[0] - m[1] + m[2] + m[5])


def _kernel(x_hbm, wqkv_hbm, wo_hbm, wg_hbm, wu_hbm, wd_hbm, out_hbm,
            x_v, wqkv_v, wo_v, wg_v, wu_v, wd_v,
            tmp, wq_t, wo_t, ga, gt, wds, res, xn1, rb, xt, rbuf, macc,
            q_s, k_s, v_s, o_s, out_v,
            sem_x, sem_a, sem_g, sem_d, sem_o):
    def cols(i, n):
        return pl.ds(i * n if isinstance(i, int) else pl.multiple_of(i * n, LANES), n)

    X_PARTS = ((0, 1), (1, 2), (2, NB))
    GU_PARTS = ((0, 1), (1, 2), (2, 4), (4, 6))
    D_PARTS = ((0, NS // 2), (NS // 2, NS))

    def cp_x(p):
        c = pl.ds(X_PARTS[p][0] * TB, (X_PARTS[p][1] - X_PARTS[p][0]) * TB)
        return pltpu.make_async_copy(x_hbm.at[:, c], x_v.at[:, c], sem_x.at[p])

    cp_qkv = pltpu.make_async_copy(wqkv_hbm, wqkv_v, sem_a.at[0])
    cp_o = pltpu.make_async_copy(wo_hbm, wo_v, sem_a.at[1])

    def half_cols(half, lo, hi):
        return pl.ds(half * F2 + lo * FS, (hi - lo) * FS)

    def cp_gu(p):
        return [pltpu.make_async_copy(src.at[:, half_cols(half, *GU_PARTS[p])],
                                      dst.at[:, half_cols(half, *GU_PARTS[p])], sem_g.at[2 * j + half, p])
                for j, (src, dst) in enumerate(((wg_hbm, wg_v), (wu_hbm, wu_v))) for half in range(2)]

    def cp_d(p):
        return [pltpu.make_async_copy(wd_hbm.at[:, half_cols(half, *D_PARTS[p])],
                                      wd_v.at[:, half_cols(half, *D_PARTS[p])], sem_d.at[half, p])
                for half in range(2)]

    def cp_out(t):
        return pltpu.make_async_copy(out_v.at[:, cols(t, TB)], out_hbm.at[:, cols(t, TB)], sem_o.at[t])

    scale = np.float32(DH ** -0.5)

    def prep_qkv():
        for j in range(NT5):
            kw = min(LANES, D - j * LANES)
            tmp[j, :, 0:kw] = wqkv_v[j * LANES:j * LANES + kw, :].astype(f32).T
        for g in range(NG):
            for p in range(3):
                for d in range(0, DH, 2):
                    r = (g * 3 + p) * GR + d * HG
                    src = p * D + g * GR + d
                    for j in range(NT5):
                        kw = min(LANES, D - j * LANES)
                        two = jnp.concatenate(
                            [tmp[j, pl.ds(src + e, HG, stride=DH), 0:kw] for e in range(2)], axis=0)
                        wq_t[r:r + 2 * HG, j * LANES:j * LANES + kw] = two.astype(bf16)

    def prep_wo():
        for j in range(NT5):
            nw = min(LANES, D - j * LANES)
            tmp[j, 0:D, 0:nw] = wo_v[:, j * LANES:j * LANES + nw].astype(f32)
            perm = jnp.concatenate(
                [tmp[j, pl.ds(g * GR + d, HG, stride=DH), 0:nw] for g in range(NG) for d in range(DH)],
                axis=0)
            wo_t[j * LANES:j * LANES + nw, :] = perm.T.astype(bf16)

    def prep_gu(s):
        for j, w_v in enumerate((wg_v, wu_v)):
            wa = w_v[:, cols(s, FS)].T
            wb = w_v[:, cols(NS + s, FS)].T
            rows = slice(j * FS, (j + 1) * FS)
            quads = [w[:, q * KH:(q + 1) * KH].astype(f32) for w in (wa, wb) for q in range(2)]
            for k, a in enumerate(_strassen_lhs(*quads)):
                ga[s, k, rows, :] = a.astype(bf16)
            gt[s, 0, rows, :] = wa[:, 2 * KH:]
            gt[s, 1, rows, :] = wb[:, 2 * KH:]

    def prep_d(s):
        ca, cb = cols(s, FS), cols(NS + s, FS)
        quads = [wd_v[0:D2, ca], wd_v[0:D2, cb], wd_v[D2:D, ca], wd_v[D2:D, cb]]
        for k, a in enumerate(_strassen_lhs(*[q.astype(f32) for q in quads])):
            wds[k, :, ca] = a.astype(bf16)

    def load_x(t):
        res[:, cols(t, TB)] = x_v[:, cols(t, TB)].astype(f32)

    def ln1(b):
        xn1[...] = _layernorm_t(res[:, cols(b % NB, TB)]).astype(bf16)

    def qkv(b, g):
        if 'q' in ABL: return
        out = _dot(wq_t[g * 3 * GR:(g + 1) * 3 * GR, :], xn1[...])
        keep = (b % NB) > 0
        n = GR // 2 if PACK else GR
        rows = slice(g * n, (g + 1) * n)
        k_s[rows, 0:LANES] = jnp.where(keep, k_s[rows, TB:TB + LANES], 0)
        v_s[rows, 0:LANES] = jnp.where(keep, v_s[rows, TB:TB + LANES], 0)
        q_s[g * GR:(g + 1) * GR, :] = out[0:GR] * scale
        if PACK:
            for dst, off in ((k_s, GR), (v_s, 2 * GR)):
                for r in range(0, GR, 2 * HG):
                    dst[g * n + r // 2:g * n + r // 2 + HG, LANES:] = pltpu.pack_elementwise(
                        [out[off + r:off + r + HG], out[off + r + HG:off + r + 2 * HG]], packed_dtype=bf16)
        else:
            k_s[rows, LANES:] = out[GR:2 * GR]
            v_s[rows, LANES:] = out[2 * GR:3 * GR]

    def heads(b, g):
        if 'h' in ABL: return
        pos = (b % NB) * TB + jax.lax.broadcasted_iota(jnp.int32, (HG, TB), 1)
        r0 = g * GR

        def windows(ref, d):
            if PACK:
                w = ref[pl.ds((r0 + d * HG) // 2, HG), :]
                sh = [(w if i == 0 else pltpu.roll(w, i * DIL, 1))[:, LANES:] for i in range(WIN)]
                return [[pltpu.unpack_elementwise(x, index=e, packed_dtype=bf16, unpacked_dtype=f32)
                         for x in sh] for e in range(2)]
            w = ref[pl.ds(r0 + d * HG, HG), :]
            return [[(w if i == 0 else pltpu.roll(w, i * DIL, 1))[:, LANES:] for i in range(WIN)]]

        dstep = 2 if PACK else 1
        logits = [None] * WIN
        for d in range(0, DH, dstep):
            for e, ks in enumerate(windows(k_s, d)):
                q = q_s[pl.ds(r0 + (d + e) * HG, HG), :]
                for w in range(WIN):
                    prod = q * ks[w]
                    logits[w] = prod if logits[w] is None else logits[w] + prod
        for w in range(1, WIN):
            logits[w] = jnp.where(pos >= w * DIL, logits[w], np.float32(-1e9))
        m = functools.reduce(jnp.maximum, logits)
        ex = [jnp.exp(l - m) for l in logits]
        inv = 1.0 / functools.reduce(jnp.add, ex)
        a = [x * inv for x in ex]
        for d in range(0, DH, dstep):
            for e, vs in enumerate(windows(v_s, d)):
                o = functools.reduce(jnp.add, [a[w] * vs[w] for w in range(WIN)])
                o_s[pl.ds(r0 + (d + e) * HG, HG), :] = o

    def attn_out(b):
        if 'o' in ABL: return
        blk = cols(b % NB, TB)
        x1 = res[:, blk] + _dot(wo_t[...], o_s[...].astype(bf16))
        res[:, blk] = x1
        xn = _layernorm_t(x1)
        slot = b % 2
        quads = [xn[q * KH:(q + 1) * KH, t * TH:(t + 1) * TH] for q in range(2) for t in range(2)]
        for k, r in enumerate(_strassen_rhs(*quads)):
            rb[slot, k] = r.astype(bf16)
        xt[slot] = xn[2 * KH:].astype(bf16)

    def strassen_products(prod, emit, hook=lambda: None):
        m = {}
        for ks, i, comb in (((2, 4), 1, lambda: m[2] + m[4]),
                            ((3, 1), 2, lambda: m[1] + m[3]),
                            ((0, 5), 3, lambda: m[0] - m[1] + m[2] + m[5]),
                            ((6,), 0, lambda: m[0] + m[3] - m[4] + m[6])):
            for k in ks:
                m[k] = prod(k)
            if i == 0:
                hook()
            emit(i, comb())

    def gate_up(b, s, hook):
        if 'f' in ABL: return hook()
        slot = b % 2
        tails = [_dot(gt[s, half], xt[slot]) for half in range(2)]
        hq = [None] * 4

        def emit(i, c):
            full = c + tails[i // 2][:, (i % 2) * TH:(i % 2 + 1) * TH]
            hq[i] = _geglu(full[:FS], full[FS:])
        strassen_products(lambda k: _dot(ga[s, k], rb[slot, k]), emit, hook)
        for k, r in enumerate(_strassen_rhs(*hq)):
            rbuf[k, s * FS:(s + 1) * FS, :] = r.astype(bf16)

    def down(b, part):
        if 'f' in ABL: return
        t0 = 2 * (b % NB)

        def emit(i, c):
            rows = slice((i // 2) * D2, (i // 2 + 1) * D2)
            dst = cols(t0 + i % 2, TH)
            y = res[rows, dst] + c
            res[rows, dst] = y
            out_v[rows, dst] = y.astype(bf16)
        strassen_products(lambda k: _dot(wds[k], rbuf[k]), emit)

    WAITALL = int(os.environ.get('WAITALL', 0))
    if WAITALL:
        allc = [cp_x(0), cp_qkv, cp_o, cp_x(1)] + cp_gu(0) + cp_gu(1) + cp_gu(2) + cp_gu(3) + [cp_x(2)] + cp_d(0) + cp_d(1)
        for i0 in range(0, len(allc), WAITALL):
            for cp in allc[i0:i0 + WAITALL]:
                cp.start()
            for cp in allc[max(i0 - WAITALL, 0):i0]:
                cp.wait()
        for cp in allc[i0:i0 + WAITALL]:
            cp.wait()

    def sync(done, launch=()):
        if WAITALL: return
        for cp in done:
            cp.wait()
        for cp in launch:
            cp.start()

    def step(i, first=False, last=False):
        nxt = not last
        half = NS // 2
        syncs = {0: (cp_gu(2), [cp_x(2)] + cp_d(0)), 2: (cp_gu(3), cp_d(1)),
                 4: ([cp_x(2)] + cp_d(0), []), 5: (cp_d(1), [])} if first else {}
        if first:
            sync(cp_gu(1), cp_gu(3))
            prep_gu(1)
        if nxt:
            ln1(i + 1)
        for s in range(NS):
            gate_up(i, s, lambda: sync(*syncs.get(s, ([], []))))
            if first:
                if s < NS - 2:
                    prep_gu(s + 2)
                if s == NS - 2:
                    for t in range(2, NB):
                        load_x(t)
                if s >= NS - 2:
                    for ss in range(half):
                        prep_d((s - NS + 2) * half + ss)
            if nxt:
                for g in range(NG):
                    if HPOS[g] == s:
                        qkv(i + 1, g)
                        heads(i + 1, g)
                if s == NS - 1:
                    attn_out(i + 1)
        down(i, 0)
        if isinstance(i, int):
            if i >= NB:
                cp_out(i - NB).start()
        else:
            @pl.when((i >= NB) & (i < NBLK) & (int(os.environ.get('EXTRA', 0)) >= 0))
            def _():
                cp_out(jnp.maximum(i - NB, 0)).start()

    sync([], [cp_x(0), cp_qkv, cp_o, cp_x(1)] + cp_gu(0))
    k_s[:, TB:] = jnp.zeros((k_s.shape[0], LANES), k_s.dtype)
    v_s[:, TB:] = jnp.zeros((v_s.shape[0], LANES), v_s.dtype)
    sync([cp_x(0)])
    load_x(0)
    ln1(0)
    sync([cp_qkv], cp_gu(1))
    prep_qkv()
    for g in range(NG):
        qkv(0, g)
        if g < NG - 1:
            heads(0, g)
    sync([cp_o, cp_x(1)] + cp_gu(0), cp_gu(2))
    heads(0, NG - 1)
    prep_wo()
    load_x(1)
    prep_gu(0)
    attn_out(0)

    step(0, first=True)
    NOLAST = int(os.environ.get('NOLAST', 1))
    jax.lax.fori_loop(1, NBLK - 1 + NOLAST + int(os.environ.get('EXTRA', 0)), lambda i, c: (step(i), c)[1], 0)
    if not NOLAST:
        step(NBLK - 1, last=True)
    for t in range(NB):
        if int(os.environ.get('EXTRA', 0)) >= 0 or (t == NB - 1 and not NOLAST):
            cp_out(t).wait()


@jax.jit
def pallas_interleave_layers__sliding_local_dilated__glu_gated_geglu__prompt_kernel(
    A_x: jax.Array,
    A_wqkv: jax.Array,
    A_wo: jax.Array,
    B_x: jax.Array,
    B_w_gate: jax.Array,
    B_w_up: jax.Array,
    B_w_down: jax.Array,
):
    del B_x
    x_t = A_x.reshape(S, D).T
    wd_t = B_w_down.T
    hbm = pl.BlockSpec(memory_space=pl.ANY)
    kv = ((D // 2, LANES + TB), jnp.int32) if PACK else ((D, LANES + TB), f32)
    out_t = pl.pallas_call(
        _kernel,
        out_shape=jax.ShapeDtypeStruct((D, S), bf16),
        in_specs=[hbm] * 6,
        out_specs=hbm,
        scratch_shapes=[
            pltpu.VMEM((D, S), bf16),
            pltpu.VMEM((D, 3 * D), bf16),
            pltpu.VMEM((D, D), bf16),
            pltpu.VMEM((D, F), bf16),
            pltpu.VMEM((D, F), bf16),
            pltpu.VMEM((D, F), bf16),
            pltpu.VMEM((NT5, 3 * D, LANES), f32),
            pltpu.VMEM((3 * D, D), bf16),
            pltpu.VMEM((D, D), bf16),
            pltpu.VMEM((NS, 7, 2 * FS, KH), bf16),
            pltpu.VMEM((NS, 2, 2 * FS, KT), bf16),
            pltpu.VMEM((7, D2, F2), bf16),
            pltpu.VMEM((D, S), f32),
            pltpu.VMEM((D, TB), bf16),
            pltpu.VMEM((2, 7, KH, TH), bf16),
            pltpu.VMEM((2, KT, TB), bf16),
            pltpu.VMEM((7, F2, TH), bf16),
            pltpu.VMEM((7, D2, TH), f32),
            pltpu.VMEM((D, TB), f32),
            pltpu.VMEM(*kv),
            pltpu.VMEM(*kv),
            pltpu.VMEM((D, TB), f32),
            pltpu.VMEM((D, S), bf16),
            pltpu.SemaphoreType.DMA((3,)),
            pltpu.SemaphoreType.DMA((2,)),
            pltpu.SemaphoreType.DMA((4, 4)),
            pltpu.SemaphoreType.DMA((2, 2)),
            pltpu.SemaphoreType.DMA((NB,)),
        ],
        compiler_params=pltpu.CompilerParams(vmem_limit_bytes=110 * 1024 * 1024),
        name="interleave_attn_geglu",
    )(x_t, A_wqkv, A_wo, B_w_gate, B_w_up, wd_t)
    return out_t.T.reshape(1, S, D)
```

```python
import functools, os

import jax
import jax.numpy as jnp
import numpy as np
import jax.experimental.pallas as pl
import jax.experimental.pallas.tpu as pltpu

S, D, F = 2048, 576, 4608
H, DH = 32, 18
WIN, DIL = 8, 2
EPS = 1e-5
LANES = 128
TB = 256
TH = TB // 2
NB = S // TB
NBLK = 2 * NB
HG = 8
NG = H // HG
GR = HG * DH
NT5 = -(-D // LANES)
F2, D2 = F // 2, D // 2
KH = 256
KT = D - 2 * KH
NS = int(os.environ.get('NS', 6))
FS = F2 // NS
DSUB = int(os.environ.get('DSUB', 6))
PACK = int(os.environ.get('PACK', 1))
WPOS = int(os.environ.get('WPOS', 0))
LAG = 1
NR = LAG + 1
HPOS = [int(c) for c in os.environ.get('HPOS', '0124')]
bf16, f32, u32 = jnp.bfloat16, jnp.float32, jnp.uint32
NN = (((1,), (0,)), ((), ()))
ABL = os.environ.get('ABL', '')


def _dot(a, b):
    return jax.lax.dot_general(a, b, NN, preferred_element_type=f32)


def _mean_rows(x):
    if int(os.environ.get('TREE', 0)):
        t = x.shape[1]
        x = x.reshape(9, D // 9, t).sum(axis=0) if int(os.environ.get('TREE', 0)) == 1 else x.reshape(8, 72, t).sum(axis=0)
        x = x.reshape(-1, 8, t).sum(axis=0)
    return jnp.sum(x, axis=0, keepdims=True) * np.float32(1.0 / D)


def _layernorm_t(x):
    xc = x - _mean_rows(x)
    return xc * jax.lax.rsqrt(_mean_rows(xc * xc) + EPS)


def _geglu(g, u):
    c0 = np.float32(np.sqrt(2.0 / np.pi))
    c1 = np.float32(np.sqrt(2.0 / np.pi) * 0.044715)
    inner = g * (c0 + c1 * (g * g))
    return (g * u) * (np.float32(0.5) + np.float32(0.5) * jnp.tanh(inner))


def _strassen_lhs_packed(quads):
    w = [pltpu.bitcast(q, u32) for q in quads]
    halves = [_strassen_lhs(*[pltpu.unpack_elementwise(x, index=e, packed_dtype=bf16, unpacked_dtype=f32)
                              for x in w]) for e in range(2)]
    out = [pltpu.bitcast(pltpu.pack_elementwise([lo, hi], packed_dtype=bf16), u32) for lo, hi in zip(*halves)]
    out[2], out[3] = w[0], w[3]
    return out


def _up(x):
    return pltpu.bitcast(x, bf16)


def _strassen_lhs(a11, a12, a21, a22):
    return [a11 + a22, a21 + a22, a11, a22, a11 + a12, a21 - a11, a12 - a22]


def _strassen_rhs(b11, b12, b21, b22):
    return [b11 + b22, b11, b12 - b22, b21 - b11, b22, b11 + b12, b21 + b22]


def _strassen_out(m):
    return (m[0] + m[3] - m[4] + m[6], m[2] + m[4], m[1] + m[3], m[0] - m[1] + m[2] + m[5])


def _kernel(x_hbm, wqkv_hbm, wo_hbm, wg_hbm, wu_hbm, wd_hbm, out_hbm,
            x_v, wqkv_v, wo_v, wg_v, wu_v, wd_v,
            tmp, wq_t, wo_t, ga, gt, wds, res, xn1, rb, xt, rbuf, macc,
            q_s, k_s, v_s, o_s, out_v,
            sem_x, sem_a, sem_g, sem_d, sem_o):
    def cols(i, n):
        return pl.ds(i * n if isinstance(i, int) else pl.multiple_of(i * n, LANES), n)

    def rows8(start, n):
        return pl.ds(start if isinstance(start, int) else pl.multiple_of(start, 8), n)

    X_PARTS = ((0, 1), (1, 2), (2, NB))
    GU_PARTS = ((0, 2), (2, 4), (4, 6))
    D_PARTS = ((0, NS),)

    def cp_x(p):
        c = pl.ds(X_PARTS[p][0] * TB, (X_PARTS[p][1] - X_PARTS[p][0]) * TB)
        return pltpu.make_async_copy(x_hbm.at[:, c], x_v.at[:, c], sem_x.at[p])

    cp_qkv = pltpu.make_async_copy(wqkv_hbm, wqkv_v, sem_a.at[0])
    cp_o = pltpu.make_async_copy(wo_hbm, wo_v, sem_a.at[1])

    def half_cols(half, lo, hi):
        return pl.ds(half * F2 + lo * FS, (hi - lo) * FS)

    def cp_gu(p):
        return [pltpu.make_async_copy(src.at[:, half_cols(half, *GU_PARTS[p])],
                                      dst.at[:, half_cols(half, *GU_PARTS[p])], sem_g.at[2 * j + half, p])
                for j, (src, dst) in enumerate(((wg_hbm, wg_v), (wu_hbm, wu_v))) for half in range(2)]

    def cp_d(p):
        return [pltpu.make_async_copy(wd_hbm.at[:, half_cols(half, *D_PARTS[p])],
                                      wd_v.at[:, half_cols(half, *D_PARTS[p])], sem_d.at[half, p])
                for half in range(2)]

    def cp_out(t):
        return pltpu.make_async_copy(out_v.at[:, cols(t, TB)], out_hbm.at[:, cols(t, TB)], sem_o.at[t])

    scale = np.float32(DH ** -0.5)

    def prep_qkv():
        for j in range(NT5):
            kw = min(LANES, D - j * LANES)
            tmp[j, :, 0:kw] = wqkv_v[j * LANES:j * LANES + kw, :].astype(f32).T
        for g in range(NG):
            for p in range(3):
                for d in range(0, DH, 2):
                    r = (g * 3 + p) * GR + d * HG
                    src = p * D + g * GR + d
                    for j in range(NT5):
                        kw = min(LANES, D - j * LANES)
                        two = jnp.concatenate(
                            [tmp[j, pl.ds(src + e, HG, stride=DH), 0:kw] for e in range(2)], axis=0)
                        wq_t[r:r + 2 * HG, j * LANES:j * LANES + kw] = two.astype(bf16)

    def prep_wo():
        for j in range(NT5):
            nw = min(LANES, D - j * LANES)
            tmp[j, 0:D, 0:nw] = wo_v[:, j * LANES:j * LANES + nw].astype(f32)
            perm = jnp.concatenate(
                [tmp[j, pl.ds(g * GR + d, HG, stride=DH), 0:nw] for g in range(NG) for d in range(DH)],
                axis=0)
            wo_t[j * LANES:j * LANES + nw, :] = perm.T.astype(bf16)

    def prep_gu(s):
        for j, w_v in enumerate((wg_v, wu_v)):
            for r in range(FS // LANES):
                wa = w_v[:, cols(s * (FS // LANES) + r, LANES)].T
                wb = w_v[:, cols((NS + s) * (FS // LANES) + r, LANES)].T
                rows = pl.ds((j * FS + r * LANES) // 2, LANES // 2)
                quads = [w[:, q * KH:(q + 1) * KH] for w in (wa, wb) for q in range(2)]
                for k, a in enumerate(_strassen_lhs_packed(quads)):
                    ga[s, k, rows, :] = a
                gt[s, 0, rows, :] = pltpu.bitcast(wa[:, 2 * KH:], u32)
                gt[s, 1, rows, :] = pltpu.bitcast(wb[:, 2 * KH:], u32)

    def prep_d(s):
        for r in range(FS // LANES):
            ca, cb = cols(s * (FS // LANES) + r, LANES), cols((NS + s) * (FS // LANES) + r, LANES)
            quads = [wd_v[0:D2, ca], wd_v[0:D2, cb], wd_v[D2:D, ca], wd_v[D2:D, cb]]
            for k, a in enumerate(_strassen_lhs_packed(quads)):
                wds[k, :, ca] = a

    def load_x(t):
        res[:, cols(t, TB)] = x_v[:, cols(t, TB)].astype(f32)

    def ln1(b, z=0):
        xn1[z] = _layernorm_t(res[:, cols(b % NB, TB)]).astype(bf16)

    def qkv(b, g, z=0, zp=0):
        if 'q' in ABL: return
        out = _dot(wq_t[rows8(g * 3 * GR, 3 * GR), :], xn1[z])
        keep = (b % NB) > 0
        n = GR // 2 if PACK else GR
        rows = rows8(g * n, n)
        k_s[z, rows, 0:LANES] = jnp.where(keep, k_s[zp, rows, TB:TB + LANES], 0)
        v_s[z, rows, 0:LANES] = jnp.where(keep, v_s[zp, rows, TB:TB + LANES], 0)
        q_s[z, rows8(g * GR, GR), :] = out[0:GR] * scale
        if PACK:
            for dst, off in ((k_s, GR), (v_s, 2 * GR)):
                for r in range(0, GR, 2 * HG):
                    dst[z, rows8(g * n + r // 2, HG), LANES:] = pltpu.pack_elementwise(
                        [out[off + r:off + r + HG], out[off + r + HG:off + r + 2 * HG]], packed_dtype=bf16)
        else:
            k_s[z, rows, LANES:] = out[GR:2 * GR]
            v_s[z, rows, LANES:] = out[2 * GR:3 * GR]

    def heads(b, g, z=0):
        if 'h' in ABL: return
        pos = (b % NB) * TB + jax.lax.broadcasted_iota(jnp.int32, (HG, TB), 1)
        r0 = g * GR

        def windows(ref, d):
            if PACK:
                w = ref[z, rows8(g * (GR // 2) + d * HG // 2, HG), :]
                sh = [(w if i == 0 else pltpu.roll(w, i * DIL, 1))[:, LANES:] for i in range(WIN)]
                return [[pltpu.unpack_elementwise(x, index=e, packed_dtype=bf16, unpacked_dtype=f32)
                         for x in sh] for e in range(2)]
            w = ref[z, rows8(r0 + d * HG, HG), :]
            return [[(w if i == 0 else pltpu.roll(w, i * DIL, 1))[:, LANES:] for i in range(WIN)]]

        dstep = 2 if PACK else 1
        logits = [None] * WIN
        for d in range(0, DH, dstep):
            for e, ks in enumerate(windows(k_s, d)):
                q = q_s[z, rows8(r0 + (d + e) * HG, HG), :]
                for w in range(WIN):
                    prod = q * ks[w]
                    logits[w] = prod if logits[w] is None else logits[w] + prod
        for w in range(1, WIN):
            logits[w] = jnp.where(pos >= w * DIL, logits[w], np.float32(-1e9))
        m = functools.reduce(jnp.maximum, logits)
        ex = [jnp.exp(l - m) for l in logits]
        inv = 1.0 / functools.reduce(jnp.add, ex)
        a = [x * inv for x in ex]
        for d in range(0, DH, dstep):
            for e, vs in enumerate(windows(v_s, d)):
                o = functools.reduce(jnp.add, [a[w] * vs[w] for w in range(WIN)])
                o_s[z, rows8(r0 + (d + e) * HG, HG), :] = o

    def attn_out(b, z=0):
        if 'o' in ABL: return
        blk = cols(b % NB, TB)
        x1 = res[:, blk] + _dot(wo_t[...], o_s[z].astype(bf16))
        res[:, blk] = x1
        xn = _layernorm_t(x1)
        slot = b % NR
        quads = [xn[q * KH:(q + 1) * KH, t * TH:(t + 1) * TH] for q in range(2) for t in range(2)]
        for k, r in enumerate(_strassen_rhs(*quads)):
            rb[slot, k] = r.astype(bf16)
        xt[slot] = xn[2 * KH:].astype(bf16)

    def strassen_products(prod, emit, hook=lambda: None, mid=lambda: None):
        m = {}
        for ks, i, comb in (((2, 4), 1, lambda: m[2] + m[4]),
                            ((3, 1), 2, lambda: m[1] + m[3]),
                            ((0, 5), 3, lambda: m[0] - m[1] + m[2] + m[5]),
                            ((6,), 0, lambda: m[0] + m[3] - m[4] + m[6])):
            for k in ks:
                m[k] = prod(k)
            if i == 0:
                hook()
            if i == WPOS:
                mid()
            emit(i, comb())

    def gate_up(b, s, hook):
        if 'f' in ABL: return hook()
        slot = b % NR
        tails = [_dot(_up(gt[s, half]), xt[slot]) for half in range(2)]
        hq = [None] * 4

        def emit(i, c):
            full = c + tails[i // 2][:, (i % 2) * TH:(i % 2 + 1) * TH]
            hq[i] = _geglu(full[:FS], full[FS:])
        strassen_products(lambda k: _dot(_up(ga[s, k]), rb[slot, k]), emit, hook)
        for k, r in enumerate(_strassen_rhs(*hq)):
            rbuf[k, cols(s, FS), :] = r.astype(bf16)

    def down(b, part):
        if 'f' in ABL: return
        t0 = 2 * (b % NB)

        def emit(i, c):
            rows = slice((i // 2) * D2, (i // 2 + 1) * D2)
            dst = cols(t0 + i % 2, TH)
            y = res[rows, dst] + c
            res[rows, dst] = y
            out_v[rows, dst] = y.astype(bf16)
        strassen_products(lambda k: _dot(_up(wds[k]), rbuf[k]), emit, mid=part)

    def sync(done, launch=()):
        for cp in done:
            cp.wait()
        for cp in launch:
            cp.start()

    def step(i, attn):
        b = i + LAG
        if attn:
            ln1(b)
        for s in range(NS):
            gate_up(i, s, lambda: None)
            if attn:
                for g in range(NG):
                    if HPOS[g] == s:
                        qkv(b, g)
                        heads(b, g)
                if s == NS - 1 and WPOS == 0:
                    attn_out(b)
        down(i, (lambda: attn_out(b)) if attn and WPOS else (lambda: None))

        @pl.when(i >= NB)
        def _():
            cp_out(jnp.maximum(i - NB, 0)).start()

    sync([], [cp_x(0), cp_qkv, cp_o, cp_x(1)] + cp_gu(0))
    k_s[0, :, TB:] = jnp.zeros((k_s.shape[1], LANES), k_s.dtype)
    v_s[0, :, TB:] = jnp.zeros((v_s.shape[1], LANES), v_s.dtype)
    sync([cp_x(0)])
    load_x(0)
    ln1(0, 1)
    sync([cp_qkv], cp_gu(1))
    prep_qkv()
    for g in range(NG):
        qkv(0, g, 1, 0)
        if g < NG - 1:
            heads(0, g, 1)
    sync([cp_o, cp_x(1)], cp_gu(2))
    heads(0, NG - 1, 1)
    prep_wo()
    load_x(1)
    attn_out(0, 1)
    ln1(1, 0)
    sync(cp_gu(0), [cp_x(2)] + cp_d(0))
    prep_gu(0)

    def first(s, carry):
        for p in range(1, len(GU_PARTS)):
            @pl.when(s + 1 == GU_PARTS[p][0])
            def _():
                sync(cp_gu(p))
        gate_up(0, s, lambda: None)
        prep_gu(jnp.minimum(s + 1, NS - 1))
        g = jnp.minimum(s, NG - 1)
        qkv(1, g, 0, 1)
        heads(1, g, 0)
        return carry
    jax.lax.fori_loop(0, NS - 1, first, 0)
    sync([cp_x(2)] + cp_d(0))
    gate_up(0, NS - 1, lambda: None)
    for t in range(2, NB):
        load_x(t)
    for s in range(NS):
        prep_d(s)
    attn_out(1, 0)
    down(0, lambda: None)

    EXTRA = int(os.environ.get('EXTRA', 0))
    jax.lax.fori_loop(1, NBLK - LAG + EXTRA, lambda i, c: (step(i, True), c)[1], 0)
    jax.lax.fori_loop(NBLK - LAG, NBLK, lambda i, c: (step(i, False), c)[1], 0,
                      unroll=bool(int(os.environ.get('UNROLL', 1))))
    for t in range(NB):
        cp_out(t).wait()


@jax.jit
def pallas_interleave_layers__sliding_local_dilated__glu_gated_geglu__prompt_kernel(
    A_x: jax.Array,
    A_wqkv: jax.Array,
    A_wo: jax.Array,
    B_x: jax.Array,
    B_w_gate: jax.Array,
    B_w_up: jax.Array,
    B_w_down: jax.Array,
):
    del B_x
    x_t = A_x.reshape(S, D).T
    wd_t = B_w_down.T
    hbm = pl.BlockSpec(memory_space=pl.ANY)
    kv = ((2, D // 2, LANES + TB), jnp.int32) if PACK else ((2, D, LANES + TB), f32)
    out_t = pl.pallas_call(
        _kernel,
        out_shape=jax.ShapeDtypeStruct((D, S), bf16),
        in_specs=[hbm] * 6,
        out_specs=hbm,
        scratch_shapes=[
            pltpu.VMEM((D, S), bf16),
            pltpu.VMEM((D, 3 * D), bf16),
            pltpu.VMEM((D, D), bf16),
            pltpu.VMEM((D, F), bf16),
            pltpu.VMEM((D, F), bf16),
            pltpu.VMEM((D, F), bf16),
            pltpu.VMEM((NT5, 3 * D, LANES), f32),
            pltpu.VMEM((3 * D, D), bf16),
            pltpu.VMEM((D, D), bf16),
            pltpu.VMEM((NS, 7, FS, KH), u32),
            pltpu.VMEM((NS, 2, FS, KT), u32),
            pltpu.VMEM((7, D2 // 2, F2), u32),
            pltpu.VMEM((D, S), f32),
            pltpu.VMEM((2, D, TB), bf16),
            pltpu.VMEM((NR, 7, KH, TH), bf16),
            pltpu.VMEM((NR, KT, TB), bf16),
            pltpu.VMEM((7, F2, TH), bf16),
            pltpu.VMEM((7, D2, TH), f32),
            pltpu.VMEM((2, D, TB), f32),
            pltpu.VMEM(*kv),
            pltpu.VMEM(*kv),
            pltpu.VMEM((2, D, TB), f32),
            pltpu.VMEM((D, S), bf16),
            pltpu.SemaphoreType.DMA((3,)),
            pltpu.SemaphoreType.DMA((2,)),
            pltpu.SemaphoreType.DMA((4, 4)),
            pltpu.SemaphoreType.DMA((2, 1)),
            pltpu.SemaphoreType.DMA((NB,)),
        ],
        compiler_params=pltpu.CompilerParams(vmem_limit_bytes=110 * 1024 * 1024),
        name="interleave_attn_geglu",
    )(x_t, A_wqkv, A_wo, B_w_gate, B_w_up, wd_t)
    return out_t.T.reshape(1, S, D)
```

```python
import functools

import jax
import jax.numpy as jnp
import numpy as np
import jax.experimental.pallas as pl
import jax.experimental.pallas.tpu as pltpu

S, D, F = 2048, 576, 4608
H, DH = 32, 18
WIN, DIL = 8, 2
EPS = 1e-5
LANES = 128
TB = 256
TH = TB // 2
NB = S // TB
NBLK = 2 * NB
HG = 8
NG = H // HG
GR = HG * DH
NT5 = -(-D // LANES)
F2, D2 = F // 2, D // 2
KH = 256
KT = D - 2 * KH
NS = 6
FS = F2 // NS
PACK = 1
WPOS = 0
LAG = 1
NR = LAG + 1
HPOS = (0, 2, 2, 4)
bf16, f32, u32 = jnp.bfloat16, jnp.float32, jnp.uint32
NN = (((1,), (0,)), ((), ()))


def _dot(a, b):
    return jax.lax.dot_general(a, b, NN, preferred_element_type=f32)


def _mean_rows(x):
    return jnp.sum(x, axis=0, keepdims=True) * np.float32(1.0 / D)


def _layernorm_t(x):
    xc = x - _mean_rows(x)
    return xc * jax.lax.rsqrt(_mean_rows(xc * xc) + EPS)


def _geglu(g, u):
    c0 = np.float32(np.sqrt(2.0 / np.pi))
    c1 = np.float32(np.sqrt(2.0 / np.pi) * 0.044715)
    inner = g * (c0 + c1 * (g * g))
    return (g * u) * (np.float32(0.5) + np.float32(0.5) * jnp.tanh(inner))


def _strassen_lhs_packed(quads):
    w = [pltpu.bitcast(q, u32) for q in quads]
    halves = [_strassen_lhs(*[pltpu.unpack_elementwise(x, index=e, packed_dtype=bf16, unpacked_dtype=f32)
                              for x in w]) for e in range(2)]
    out = [pltpu.bitcast(pltpu.pack_elementwise([lo, hi], packed_dtype=bf16), u32) for lo, hi in zip(*halves)]
    out[2], out[3] = w[0], w[3]
    return out


def _up(x):
    return pltpu.bitcast(x, bf16)


def _strassen_lhs(a11, a12, a21, a22):
    return [a11 + a22, a21 + a22, a11, a22, a11 + a12, a21 - a11, a12 - a22]


def _strassen_rhs(b11, b12, b21, b22):
    return [b11 + b22, b11, b12 - b22, b21 - b11, b22, b11 + b12, b21 + b22]


def _strassen_out(m):
    return (m[0] + m[3] - m[4] + m[6], m[2] + m[4], m[1] + m[3], m[0] - m[1] + m[2] + m[5])


def _kernel(x_hbm, wqkv_hbm, wo_hbm, wg_hbm, wu_hbm, wd_hbm, out_hbm,
            x_v, wqkv_v, wo_v, wg_v, wu_v, wd_v,
            tmp, wq_t, wo_t, ga, gt, wds, res, xn1, rb, xt, rbuf, macc,
            q_s, k_s, v_s, o_s, out_v,
            sem_x, sem_a, sem_g, sem_d, sem_o):
    def cols(i, n):
        return pl.ds(i * n if isinstance(i, int) else pl.multiple_of(i * n, LANES), n)

    def rows8(start, n):
        return pl.ds(start if isinstance(start, int) else pl.multiple_of(start, 8), n)

    X_PARTS = ((0, 1), (1, 2), (2, NB))
    GU_PARTS = ((0, 1), (1, 3), (3, 6))
    D_PARTS = ((0, NS),)

    def cp_x(p):
        c = pl.ds(X_PARTS[p][0] * TB, (X_PARTS[p][1] - X_PARTS[p][0]) * TB)
        return pltpu.make_async_copy(x_hbm.at[:, c], x_v.at[:, c], sem_x.at[p])

    cp_qkv = pltpu.make_async_copy(wqkv_hbm, wqkv_v, sem_a.at[0])
    cp_o = pltpu.make_async_copy(wo_hbm, wo_v, sem_a.at[1])

    def half_cols(half, lo, hi):
        return pl.ds(half * F2 + lo * FS, (hi - lo) * FS)

    def cp_gu(p):
        return [pltpu.make_async_copy(src.at[:, half_cols(half, *GU_PARTS[p])],
                                      dst.at[:, half_cols(half, *GU_PARTS[p])], sem_g.at[2 * j + half, p])
                for j, (src, dst) in enumerate(((wg_hbm, wg_v), (wu_hbm, wu_v))) for half in range(2)]

    def cp_d(p):
        return [pltpu.make_async_copy(wd_hbm.at[:, half_cols(half, *D_PARTS[p])],
                                      wd_v.at[:, half_cols(half, *D_PARTS[p])], sem_d.at[half, p])
                for half in range(2)]

    def cp_out(t):
        return pltpu.make_async_copy(out_v.at[:, cols(t, TB)], out_hbm.at[:, cols(t, TB)], sem_o.at[t])

    scale = np.float32(DH ** -0.5)

    def prep_qkv():
        for j in range(NT5):
            kw = min(LANES, D - j * LANES)
            tmp[j, :, 0:kw] = wqkv_v[j * LANES:j * LANES + kw, :].astype(f32).T
        for g in range(NG):
            for p in range(3):
                for d in range(0, DH, 2):
                    r = (g * 3 + p) * GR + d * HG
                    src = p * D + g * GR + d
                    for j in range(NT5):
                        kw = min(LANES, D - j * LANES)
                        two = jnp.concatenate(
                            [tmp[j, pl.ds(src + e, HG, stride=DH), 0:kw] for e in range(2)], axis=0)
                        wq_t[r:r + 2 * HG, j * LANES:j * LANES + kw] = two.astype(bf16)

    def prep_wo():
        for j in range(NT5):
            nw = min(LANES, D - j * LANES)
            tmp[j, 0:D, 0:nw] = wo_v[:, j * LANES:j * LANES + nw].astype(f32)
            perm = jnp.concatenate(
                [tmp[j, pl.ds(g * GR + d, HG, stride=DH), 0:nw] for g in range(NG) for d in range(DH)],
                axis=0)
            wo_t[j * LANES:j * LANES + nw, :] = perm.T.astype(bf16)

    def prep_gu(s):
        for j, w_v in enumerate((wg_v, wu_v)):
            for r in range(FS // LANES):
                wa = w_v[:, cols(s * (FS // LANES) + r, LANES)].T
                wb = w_v[:, cols((NS + s) * (FS // LANES) + r, LANES)].T
                rows = pl.ds((j * FS + r * LANES) // 2, LANES // 2)
                quads = [w[:, q * KH:(q + 1) * KH] for w in (wa, wb) for q in range(2)]
                for k, a in enumerate(_strassen_lhs_packed(quads)):
                    ga[s, k, rows, :] = a
                gt[s, 0, rows, :] = pltpu.bitcast(wa[:, 2 * KH:], u32)
                gt[s, 1, rows, :] = pltpu.bitcast(wb[:, 2 * KH:], u32)

    def prep_d(s):
        for r in range(FS // LANES):
            ca, cb = cols(s * (FS // LANES) + r, LANES), cols((NS + s) * (FS // LANES) + r, LANES)
            quads = [wd_v[0:D2, ca], wd_v[0:D2, cb], wd_v[D2:D, ca], wd_v[D2:D, cb]]
            for k, a in enumerate(_strassen_lhs_packed(quads)):
                wds[k, :, ca] = a

    def load_x(t):
        res[:, cols(t, TB)] = x_v[:, cols(t, TB)].astype(f32)

    def ln1(b, z=0):
        xn1[z] = _layernorm_t(res[:, cols(b % NB, TB)]).astype(bf16)

    def qkv(b, g, z=0, zp=0):
        out = _dot(wq_t[rows8(g * 3 * GR, 3 * GR), :], xn1[z])
        keep = (b % NB) > 0
        n = GR // 2 if PACK else GR
        rows = rows8(g * n, n)
        k_s[z, rows, 0:LANES] = jnp.where(keep, k_s[zp, rows, TB:TB + LANES], 0)
        v_s[z, rows, 0:LANES] = jnp.where(keep, v_s[zp, rows, TB:TB + LANES], 0)
        q_s[z, rows8(g * GR, GR), :] = out[0:GR] * scale
        if PACK:
            for dst, off in ((k_s, GR), (v_s, 2 * GR)):
                for r in range(0, GR, 2 * HG):
                    dst[z, rows8(g * n + r // 2, HG), LANES:] = pltpu.pack_elementwise(
                        [out[off + r:off + r + HG], out[off + r + HG:off + r + 2 * HG]], packed_dtype=bf16)
        else:
            k_s[z, rows, LANES:] = out[GR:2 * GR]
            v_s[z, rows, LANES:] = out[2 * GR:3 * GR]

    def heads(b, g, z=0):
        pos = (b % NB) * TB + jax.lax.broadcasted_iota(jnp.int32, (HG, TB), 1)
        r0 = g * GR

        def windows(ref, d):
            if PACK:
                w = ref[z, rows8(g * (GR // 2) + d * HG // 2, HG), :]
                sh = [(w if i == 0 else pltpu.roll(w, i * DIL, 1))[:, LANES:] for i in range(WIN)]
                return [[pltpu.unpack_elementwise(x, index=e, packed_dtype=bf16, unpacked_dtype=f32)
                         for x in sh] for e in range(2)]
            w = ref[z, rows8(r0 + d * HG, HG), :]
            return [[(w if i == 0 else pltpu.roll(w, i * DIL, 1))[:, LANES:] for i in range(WIN)]]

        dstep = 2 if PACK else 1
        logits = [None] * WIN
        for d in range(0, DH, dstep):
            for e, ks in enumerate(windows(k_s, d)):
                q = q_s[z, rows8(r0 + (d + e) * HG, HG), :]
                for w in range(WIN):
                    prod = q * ks[w]
                    logits[w] = prod if logits[w] is None else logits[w] + prod
        for w in range(1, WIN):
            logits[w] = jnp.where(pos >= w * DIL, logits[w], np.float32(-1e9))
        m = functools.reduce(jnp.maximum, logits)
        ex = [jnp.exp(l - m) for l in logits]
        inv = 1.0 / functools.reduce(jnp.add, ex)
        a = [x * inv for x in ex]
        for d in range(0, DH, dstep):
            for e, vs in enumerate(windows(v_s, d)):
                o = functools.reduce(jnp.add, [a[w] * vs[w] for w in range(WIN)])
                o_s[z, rows8(r0 + (d + e) * HG, HG), :] = o

    def attn_out(b, z=0):
        blk = cols(b % NB, TB)
        x1 = res[:, blk] + _dot(wo_t[...], o_s[z].astype(bf16))
        res[:, blk] = x1
        xn = _layernorm_t(x1)
        slot = b % NR
        quads = [xn[q * KH:(q + 1) * KH, t * TH:(t + 1) * TH] for q in range(2) for t in range(2)]
        for k, r in enumerate(_strassen_rhs(*quads)):
            rb[slot, k] = r.astype(bf16)
        xt[slot] = xn[2 * KH:].astype(bf16)

    def strassen_products(prod, emit, hook=lambda: None, mid=lambda: None):
        m = {}
        for ks, i, comb in (((2, 4), 1, lambda: m[2] + m[4]),
                            ((3, 1), 2, lambda: m[1] + m[3]),
                            ((0, 5), 3, lambda: m[0] - m[1] + m[2] + m[5]),
                            ((6,), 0, lambda: m[0] + m[3] - m[4] + m[6])):
            for k in ks:
                m[k] = prod(k)
            if i == 0:
                hook()
            if i == WPOS:
                mid()
            emit(i, comb())

    def gate_up(b, s, hook):
        slot = b % NR
        tails = [_dot(_up(gt[s, half]), xt[slot]) for half in range(2)]
        hq = [None] * 4

        def emit(i, c):
            full = c + tails[i // 2][:, (i % 2) * TH:(i % 2 + 1) * TH]
            hq[i] = _geglu(full[:FS], full[FS:])
        strassen_products(lambda k: _dot(_up(ga[s, k]), rb[slot, k]), emit, hook)
        for k, r in enumerate(_strassen_rhs(*hq)):
            rbuf[k, cols(s, FS), :] = r.astype(bf16)

    def down(b, part):
        t0 = 2 * (b % NB)

        def emit(i, c):
            rows = slice((i // 2) * D2, (i // 2 + 1) * D2)
            dst = cols(t0 + i % 2, TH)
            y = res[rows, dst] + c
            res[rows, dst] = y
            out_v[rows, dst] = y.astype(bf16)
        strassen_products(lambda k: _dot(_up(wds[k]), rbuf[k]), emit, mid=part)

    def sync(done, launch=()):
        for cp in done:
            cp.wait()
        for cp in launch:
            cp.start()

    def step(i, attn):
        b = i + LAG
        if attn:
            ln1(b)
        for s in range(NS):
            gate_up(i, s, lambda: None)
            if attn:
                for g in range(NG):
                    if HPOS[g] == s:
                        qkv(b, g)
                        heads(b, g)
                if s == NS - 1 and WPOS == 0:
                    attn_out(b)
        down(i, (lambda: attn_out(b)) if attn and WPOS else (lambda: None))

        @pl.when(i >= NB)
        def _():
            cp_out(jnp.maximum(i - NB, 0)).start()

    sync([], [cp_x(0), cp_qkv, cp_o, cp_x(1)] + cp_gu(0))
    k_s[0, :, TB:] = jnp.zeros((k_s.shape[1], LANES), k_s.dtype)
    v_s[0, :, TB:] = jnp.zeros((v_s.shape[1], LANES), v_s.dtype)
    sync([cp_x(0)])
    load_x(0)
    ln1(0, 1)
    sync([cp_qkv], cp_gu(1))
    prep_qkv()
    for g in range(NG):
        qkv(0, g, 1, 0)
        if g < NG - 1:
            heads(0, g, 1)
    sync([cp_o, cp_x(1)] + cp_gu(0), cp_gu(2) + [cp_x(2)] + cp_d(0))
    heads(0, NG - 1, 1)
    prep_wo()
    load_x(1)
    prep_gu(0)
    attn_out(0, 1)
    ln1(1, 0)

    def first(s, carry):
        for p in range(1, len(GU_PARTS)):
            @pl.when(s + 1 == GU_PARTS[p][0])
            def _():
                sync(cp_gu(p))
        g = jnp.minimum(s, NG - 1)
        for o in 'pqgh':
            if o == 'g': gate_up(0, s, lambda: None)
            if o == 'p': prep_gu(jnp.minimum(s + 1, NS - 1))
            if o == 'q': qkv(1, g, 0, 1)
            if o == 'h': heads(1, g, 0)
        return carry
    jax.lax.fori_loop(0, NS - 1, first, 0)
    sync([cp_x(2)] + cp_d(0))
    gate_up(0, NS - 1, lambda: None)
    for t in range(2, NB):
        load_x(t)
    for s in range(NS):
        prep_d(s)
    attn_out(1, 0)
    down(0, lambda: None)

    jax.lax.fori_loop(1, NBLK - LAG, lambda i, c: (step(i, True), c)[1], 0)
    jax.lax.fori_loop(NBLK - LAG, NBLK, lambda i, c: (step(i, False), c)[1], 0,
                      unroll=True)
    for t in range(NB):
        cp_out(t).wait()


@jax.jit
def pallas_interleave_layers__sliding_local_dilated__glu_gated_geglu__prompt_kernel(
    A_x: jax.Array,
    A_wqkv: jax.Array,
    A_wo: jax.Array,
    B_x: jax.Array,
    B_w_gate: jax.Array,
    B_w_up: jax.Array,
    B_w_down: jax.Array,
):
    del B_x
    x_t = A_x.reshape(S, D).T
    wd_t = B_w_down.T
    hbm = pl.BlockSpec(memory_space=pl.ANY)
    kv = ((2, D // 2, LANES + TB), jnp.int32) if PACK else ((2, D, LANES + TB), f32)
    out_t = pl.pallas_call(
        _kernel,
        out_shape=jax.ShapeDtypeStruct((D, S), bf16),
        in_specs=[hbm] * 6,
        out_specs=hbm,
        scratch_shapes=[
            pltpu.VMEM((D, S), bf16),
            pltpu.VMEM((D, 3 * D), bf16),
            pltpu.VMEM((D, D), bf16),
            pltpu.VMEM((D, F), bf16),
            pltpu.VMEM((D, F), bf16),
            pltpu.VMEM((D, F), bf16),
            pltpu.VMEM((NT5, 3 * D, LANES), f32),
            pltpu.VMEM((3 * D, D), bf16),
            pltpu.VMEM((D, D), bf16),
            pltpu.VMEM((NS, 7, FS, KH), u32),
            pltpu.VMEM((NS, 2, FS, KT), u32),
            pltpu.VMEM((7, D2 // 2, F2), u32),
            pltpu.VMEM((D, S), f32),
            pltpu.VMEM((2, D, TB), bf16),
            pltpu.VMEM((NR, 7, KH, TH), bf16),
            pltpu.VMEM((NR, KT, TB), bf16),
            pltpu.VMEM((7, F2, TH), bf16),
            pltpu.VMEM((7, D2, TH), f32),
            pltpu.VMEM((2, D, TB), f32),
            pltpu.VMEM(*kv),
            pltpu.VMEM(*kv),
            pltpu.VMEM((2, D, TB), f32),
            pltpu.VMEM((D, S), bf16),
            pltpu.SemaphoreType.DMA((3,)),
            pltpu.SemaphoreType.DMA((2,)),
            pltpu.SemaphoreType.DMA((4, 4)),
            pltpu.SemaphoreType.DMA((2, 1)),
            pltpu.SemaphoreType.DMA((NB,)),
        ],
        compiler_params=pltpu.CompilerParams(vmem_limit_bytes=110 * 1024 * 1024),
        name="interleave_attn_geglu",
    )(x_t, A_wqkv, A_wo, B_w_gate, B_w_up, wd_t)
    return out_t.T.reshape(1, S, D)
```
